```python
import jax
import jax.numpy as jnp

def _softmax(x, axis=-1):
    return jax.nn.softmax(x, axis=axis)
def _gelu(x):
    return jax.nn.gelu(x, approximate=True)
def _silu(x):
    return jax.nn.silu(x)
def _sigmoid(x):
    return jax.nn.sigmoid(x)
def _layernorm(x, axis=-1, eps=1e-5):
    m = jnp.mean(x, axis=axis, keepdims=True)
    v = jnp.var(x, axis=axis, keepdims=True)
    return (x - m) / jnp.sqrt(v + eps)
def _scatter_add(tgt, idx, src, axis=0):
    return tgt.at[idx].add(src)
def _segment_sum(src, seg, n):
    return jax.ops.segment_sum(src, seg, n)
class _Rng:
    def __init__(self, key):
        self._k = key
    def _next(self):
        self._k, sub = jax.random.split(self._k)
        return sub
    def normal(self, shape):
        return jax.random.normal(self._next(), shape, dtype=jnp.bfloat16)
    def randint(self, lo, hi, shape):
        return jax.random.randint(self._next(), shape, lo, hi, dtype=jnp.int32)
    def uniform(self, shape, lo=0.0, hi=1.0):
        return jax.random.uniform(self._next(), shape, jnp.bfloat16, lo, hi)
    def permutation(self, n):
        return jax.random.permutation(self._next(), n)


kernel_name = 'interleave_layers__sliding_block_cached__dense_activation_gelu__decode'

def _fwd_setup_inputs():
    _rng = _Rng(jax.random.key(int.from_bytes(__import__("os").urandom(4), "little")))
    _w = (lambda a: (lambda t: t.astype(jnp.bfloat16) if jnp.issubdtype(t.dtype, jnp.floating) else t)(jnp.asarray(a)))
    def _A_setup():
        B, Sq, D = 2, 1, 512
        Hq, Hkv, Sk, Dh = 32, 8, 32768, 128
        assert Hq % Hkv == 0, (Hq, Hkv)
        return {
            "x": _w((lambda *s: _rng.normal(s) * 0.05)(B, Sq, D)),
            "k_cache": _w((lambda *s: _rng.normal(s) * 0.05)(B, Hkv, Sk, Dh)),
            "v_cache": _w((lambda *s: _rng.normal(s) * 0.05)(B, Hkv, Sk, Dh)),
            "wq": _w((lambda *s: _rng.normal(s) * 0.05)(D, Hq * Dh) * (D ** -0.5)),
            "wo": _w((lambda *s: _rng.normal(s) * 0.05)(Hq * Dh, D) * ((Hq * Dh) ** -0.5)),
        }
    _A_in = _A_setup()

    def _B_setup():
        B, S, D, F = 2, 1, 512, 1792
        return {
            "x": _w((lambda *s: _rng.normal(s) * 0.05)(B, S, D)),
            "w1": _w((lambda *s: _rng.normal(s) * 0.05)(D, F) * (D ** -0.5)),
            "b1": _w((lambda *s: _rng.normal(s) * 0.05)(F) * 0.01),
            "w2": _w((lambda *s: _rng.normal(s) * 0.05)(F, D) * (F ** -0.5)),
            "b2": _w((lambda *s: _rng.normal(s) * 0.05)(D) * 0.01),
        }
    _B_in = _B_setup()

    return {
        "A_x": _A_in["x"],
        "A_k_cache": _A_in["k_cache"],
        "A_v_cache": _A_in["v_cache"],
        "A_wq": _A_in["wq"],
        "A_wo": _A_in["wo"],
        "B_x": _B_in["x"],
        "B_w1": _B_in["w1"],
        "B_b1": _B_in["b1"],
        "B_w2": _B_in["w2"],
        "B_b2": _B_in["b2"],
    }

def _fwd_reference(A_x, A_k_cache, A_v_cache, A_wq, A_wo, B_x, B_w1, B_b1, B_w2, B_b2):
    def _A_ref(x, k_cache, v_cache, wq, wo):
        B, Sq, D = x.shape
        Hq, Dh = 32, 128
        Hkv, Sk = k_cache.shape[1], k_cache.shape[2]
        W = min(4096, max(256, Sk // 4))
        rep = Hq // Hkv
        q = (lambda x, *d: x.transpose(*d))((x @ wq).reshape(B, Sq, Hq, Dh), 0, 2, 1, 3)
        k = jnp.repeat(k_cache[:, :, Sk - W:, :], rep, axis=1)
        v = jnp.repeat(v_cache[:, :, Sk - W:, :], rep, axis=1)
        scores = jnp.einsum("bhqd,bhkd->bhqk", q, k) * (Dh ** -0.5)
        p = _softmax(scores, axis=-1)
        o = jnp.einsum("bhqk,bhkd->bhqd", p, v)
        return (lambda x, *d: x.transpose(*d))(o, 0, 2, 1, 3).reshape(B, Sq, Hq * Dh) @ wo

    def _B_ref(x, w1, b1, w2, b2):
        h = jnp.einsum("bsd,df->bsf", x, w1) + b1
        h = _gelu(h)
        return jnp.einsum("bsf,fd->bsd", h, w2) + b2

    x = A_x
    x = x + _A_ref(_layernorm(x, axis=-1), A_k_cache, A_v_cache, A_wq, A_wo)
    x = x + _B_ref(_layernorm(x, axis=-1), B_w1, B_b1, B_w2, B_b2)
    x = x + _A_ref(_layernorm(x, axis=-1), A_k_cache, A_v_cache, A_wq, A_wo)
    x = x + _B_ref(_layernorm(x, axis=-1), B_w1, B_b1, B_w2, B_b2)
    return x


def setup_inputs():
    _inp = _fwd_setup_inputs()
    _gk = jax.random.fold_in(jax.random.key(int.from_bytes(__import__("os").urandom(4), "little")), 2**31 - 1)
    _shapes = [[2, 1, 512]]
    _dtypes = ['bfloat16']
    _gks = jax.random.split(_gk, len(_shapes))
    _gs = [jax.random.normal(k, s, dtype=jnp.dtype(d)) * 0.05 for k, s, d in zip(_gks, _shapes, _dtypes)]
    _inp["grad_out"] = _gs[0]
    return _inp

def reference(A_x, A_k_cache, A_v_cache, A_wq, A_wo, B_w1, B_b1, B_w2, B_b2, B_x, grad_out):
    _const = dict(B_x=B_x)
    def _f(*_d):
        return _fwd_reference(**{'A_x': _d[0], 'A_k_cache': _d[1], 'A_v_cache': _d[2], 'A_wq': _d[3], 'A_wo': _d[4], 'B_w1': _d[5], 'B_b1': _d[6], 'B_w2': _d[7], 'B_b2': _d[8], **_const})
    _out, _vjp = jax.vjp(_f, A_x, A_k_cache, A_v_cache, A_wq, A_wo, B_w1, B_b1, B_w2, B_b2)
    _grads = _vjp(grad_out)
    _out0 = jnp.asarray(_out)
    return (_out0, *[jnp.asarray(_g) for _g in _grads])
```

```python
import math

import jax
import jax.numpy as jnp
from jax import lax
import jax.experimental.pallas as pl
import jax.experimental.pallas.tpu as pltpu

F32 = jnp.float32
BF16 = jnp.bfloat16

HQ, DH = 32, 128
ROWS = 112
STEP = 16
INIT = 4
TAIL = 512
LN_EPS = 1e-5
GELU_C = math.sqrt(2.0 / math.pi)
GELU_A = 0.044715

NN = (((1,), (0,)), ((), ()))
NT = (((1,), (1,)), ((), ()))
TN = (((0,), (0,)), ((), ()))


def _dot(a, b, dims):
    return lax.dot_general(a, b, dims, preferred_element_type=F32)


def _layernorm(x):
    mean = jnp.mean(x, axis=-1, keepdims=True)
    cen = x - mean
    var = jnp.mean(cen * cen, axis=-1, keepdims=True)
    rstd = 1.0 / jnp.sqrt(var + LN_EPS)
    return cen * rstd, rstd


def _layernorm_bwd(dn, n, rstd):
    m1 = jnp.mean(dn, axis=-1, keepdims=True)
    m2 = jnp.mean(dn * n, axis=-1, keepdims=True)
    return rstd * (dn - m1 - n * m2)


def _gelu(z):
    z2 = z * z
    t = jnp.tanh(GELU_C * (z + GELU_A * z2 * z))
    cdf = 0.5 * (1.0 + t)
    dcdf = 0.5 * (1.0 - t * t) * (GELU_C * (1.0 + 3.0 * GELU_A * z2))
    return z * cdf, cdf + z * dcdf


def _kernel(
    x_hbm, k_hbm, v_hbm, wq_hbm, wo_hbm, w1_hbm, b1_hbm, w2_hbm, b2_hbm, g_hbm,
    out_hbm, dx_hbm, dk_hbm, dv_hbm, dwq_hbm, dwo_hbm, dw1_hbm, db1_hbm,
    dw2_hbm, db2_hbm,
    x_v, g_v, b1_v, b2_v, out_v, dx_v, db1_v, db2_v,
    k_v, v_v, wq_v, wo_v, w1_v, w2_v,
    dk_v, dv_v, dwq_v, dwo_v, dw1_v, dw2_v,
    zero_v, q_s, do_s, o_s, dq_s, p_s, ds_s,
    rd_sem, zero_sem, wr_sem,
):
    B, HKV, SK, _ = k_hbm.shape
    W = k_v.shape[2]
    Z = SK - W
    REP = HQ // HKV
    R = B * REP
    scale = DH ** -0.5
    F = w2_hbm.shape[0]

    reads = [
        (x_hbm, x_v), (g_hbm, g_v), (b1_hbm, b1_v), (b2_hbm, b2_v),
        (wq_hbm, wq_v),
        (k_hbm.at[:, :, pl.ds(Z, W), :], k_v),
        (v_hbm.at[:, :, pl.ds(Z, W), :], v_v),
        (wo_hbm, wo_v), (w1_hbm, w1_v),
        (w2_hbm.at[pl.ds(0, F - TAIL)], w2_v.at[pl.ds(0, F - TAIL)]),
        (w2_hbm.at[pl.ds(F - TAIL, TAIL)], w2_v.at[pl.ds(F - TAIL, TAIL)]),
    ]
    reads = [pltpu.make_async_copy(s, d, rd_sem.at[i])
             for i, (s, d) in enumerate(reads)]
    for r in reads:
        r.start()
    zero_v[...] = jnp.zeros(zero_v.shape, zero_v.dtype)
    for r in reads[:-1]:
        r.wait()

    ZC = Z // ROWS
    NZ = B * ZC

    def zero_copy(dst, j):
        rows = pl.ds(pl.multiple_of((j % ZC) * ROWS, ROWS), ROWS)
        return pltpu.make_async_copy(
            zero_v, dst.at[j // ZC, :, rows, :], zero_sem)

    def fill(first, n):
        def run(dst, base):
            def body(j, carry):
                zero_copy(dst, j).start()
                return carry
            lax.fori_loop(base, base + n, body, 0)

        if isinstance(first, int):
            if first < NZ:
                assert first + n <= NZ
                run(dk_hbm, first)
            else:
                assert first + n <= 2 * NZ
                run(dv_hbm, first - NZ)
        else:
            pl.when(first < NZ)(lambda: run(dk_hbm, first))
            pl.when(first >= NZ)(lambda: run(dv_hbm, first - NZ))

    issued = [0]

    def top_up(n=STEP):
        for _ in range(n // STEP):
            fill(issued[0], STEP)
            issued[0] += STEP

    def head_loop(body, n=STEP):
        base = issued[0]

        def step(h, carry):
            for i in range(n // STEP):
                fill(base + h * n + i * STEP, STEP)
            body(h)
            return carry
        lax.fori_loop(0, HKV, step, 0)
        issued[0] = base + HKV * n

    top_up(INIT * STEP)
    reads[-1].wait()

    def row_ids(width):
        return lax.broadcasted_iota(jnp.int32, (R, width), 0)

    def load_rows(ref):
        width = ref.shape[-1]
        rows = ref[...].astype(F32)
        x = jnp.broadcast_to(rows[0:1], (R, width))
        for b in range(1, B):
            xb = jnp.broadcast_to(rows[b:b + 1], (R, width))
            x = jnp.where(row_ids(width) % B == b, xb, x)
        return x

    def store_rows(ref, x):
        ref[...] = x[:B].astype(ref.dtype)

    def split_heads(x):
        head = row_ids(DH) // B
        tiles = []
        for h in range(HKV):
            t = x[:, h * REP * DH:(h * REP + 1) * DH]
            for r in range(1, REP):
                c = (h * REP + r) * DH
                t = jnp.where(head == r, x[:, c:c + DH], t)
            tiles.append(t)
        return tiles

    def sum_heads(x):
        s = B
        while s < R:
            x = x + pltpu.roll(x, s, axis=0)
            s *= 2
        return x

    def merge_heads(ref, layer):
        head = row_ids(DH) // B
        cols = []
        for h in range(HKV):
            t = ref[h, layer]
            for r in range(REP):
                cols.append(sum_heads(jnp.where(head == r, t, 0.0)))
        return jnp.concatenate(cols, axis=1)

    def per_batch(fn):
        y = fn(0)
        for b in range(1, B):
            y = jnp.where(row_ids(y.shape[1]) % B == b, fn(b), y)
        return y

    def both_layers(a, b):
        keep = row_ids(a.shape[1]) < B
        return jnp.concatenate(
            [jnp.where(keep, a, 0.0), jnp.where(keep, b, 0.0)], axis=0
        ).astype(BF16)

    def batch_sum(a):
        keep = row_ids(a.shape[1]) < B
        return jnp.sum(jnp.where(keep, a, 0.0), axis=0, keepdims=True)

    def attn_fwd(x, layer):
        n, rstd = _layernorm(x)
        q = _dot(n.astype(BF16), wq_v[...], NN)
        for h, t in enumerate(split_heads(q)):
            q_s[h, layer] = t
        top_up()

        def body(h):
            qh = q_s[h, layer].astype(BF16)
            s = per_batch(lambda b: _dot(qh, k_v[b, h], NT)) * scale
            e = jnp.exp(s - jnp.max(s, axis=-1, keepdims=True))
            p = e / jnp.sum(e, axis=-1, keepdims=True)
            p_s[h, layer] = p
            pb = p.astype(BF16)
            o_s[h, layer] = per_batch(lambda b: _dot(pb, v_v[b, h], NN))
        head_loop(body)
        o = merge_heads(o_s, layer)
        y = _dot(o.astype(BF16), wo_v[...], NN)
        top_up()
        return x + y, (n, rstd, o)

    def attn_bwd(g, layer, saved):
        n, rstd, _ = saved
        do = _dot(g.astype(BF16), wo_v[...], NT)
        for h, t in enumerate(split_heads(do)):
            do_s[h, layer] = t
        top_up()

        def body(h):
            doh = do_s[h, layer].astype(BF16)
            dp = per_batch(lambda b: _dot(doh, v_v[b, h], NT))
            p = p_s[h, layer]
            ds = p * (dp - jnp.sum(p * dp, axis=-1, keepdims=True)) * scale
            dsb = ds.astype(BF16)
            dq_s[h, layer] = per_batch(lambda b: _dot(dsb, k_v[b, h], NN))
            if layer == 1:
                ds_s[h] = ds
                return
            batch = lax.broadcasted_iota(jnp.int32, (2 * R, DH), 0) % B

            def cache_grad(dst, lhs, rhs):
                rhs = jnp.concatenate(
                    [jnp.where(batch == b, rhs, 0.0) for b in range(B)], axis=1)
                res = _dot(lhs.astype(BF16), rhs.astype(BF16), TN)
                for b in range(B):
                    dst[b, h] = res[:, b * DH:(b + 1) * DH].astype(BF16)

            cache_grad(dk_v, jnp.concatenate([ds, ds_s[h]], axis=0),
                       jnp.concatenate([q_s[h, 0], q_s[h, 1]], axis=0))
            cache_grad(dv_v, jnp.concatenate([p, p_s[h, 1]], axis=0),
                       jnp.concatenate([do_s[h, 0], do_s[h, 1]], axis=0))
        head_loop(body, STEP if layer == 1 else 2 * STEP)
        dq = merge_heads(dq_s, layer)
        dn = _dot(dq.astype(BF16), wq_v[...], NT)
        top_up()
        return g + _layernorm_bwd(dn, n, rstd), dq

    def ffn_fwd(x):
        n, rstd = _layernorm(x)
        b1 = b1_v[...].astype(F32).reshape(1, -1)
        b2 = b2_v[...].astype(F32).reshape(1, -1)
        a, da = _gelu(_dot(n.astype(BF16), w1_v[...], NN) + b1)
        y = _dot(a.astype(BF16), w2_v[...], NN) + b2
        return x + y, (n, rstd, a, da)

    def ffn_bwd(g, saved):
        n, rstd, _, da = saved
        dz = _dot(g.astype(BF16), w2_v[...], NT) * da
        dn = _dot(dz.astype(BF16), w1_v[...], NT)
        return g + _layernorm_bwd(dn, n, rstd), dz

    x0 = load_rows(x_v)
    x1, sa0 = attn_fwd(x0, 0)
    x2, sf0 = ffn_fwd(x1)
    x3, sa1 = attn_fwd(x2, 1)
    x4, sf1 = ffn_fwd(x3)
    store_rows(out_v, x4)

    g4 = load_rows(g_v)
    g3, dz1 = ffn_bwd(g4, sf1)
    g2, dq1 = attn_bwd(g3, 1, sa1)
    g1, dz0 = ffn_bwd(g2, sf0)
    g0, dq0 = attn_bwd(g1, 0, sa0)
    store_rows(dx_v, g0)

    db1_v[...] = batch_sum(dz0 + dz1).reshape(-1).astype(BF16)
    db2_v[...] = batch_sum(g2 + g4).reshape(-1).astype(BF16)
    dwq_v[...] = _dot(both_layers(sa0[0], sa1[0]), both_layers(dq0, dq1), TN).astype(BF16)
    dwo_v[...] = _dot(both_layers(sa0[2], sa1[2]), both_layers(g1, g3), TN).astype(BF16)
    dw1_v[...] = _dot(both_layers(sf0[0], sf1[0]), both_layers(dz0, dz1), TN).astype(BF16)
    dw2_v[...] = _dot(both_layers(sf0[2], sf1[2]), both_layers(g2, g4), TN).astype(BF16)

    small = [(out_v, out_hbm), (dx_v, dx_hbm), (db1_v, db1_hbm), (db2_v, db2_hbm),
             (dwq_v, dwq_hbm), (dwo_v, dwo_hbm), (dw1_v, dw1_hbm), (dw2_v, dw2_hbm)]
    small = [pltpu.make_async_copy(s, d, wr_sem.at[i])
             for i, (s, d) in enumerate(small)]
    for c in small[:4]:
        c.start()
    top_up(2 * NZ - issued[0])

    def write_weight(i, src, dst, groups, rows, cols):
        n, m = src.shape
        src = src.reshape(groups, n // groups, m)
        dst = dst.reshape(groups, n // groups, m)

        def body(j, carry):
            r = pl.ds(pl.multiple_of(j * rows, rows), rows)
            for c in range(0, m, cols):
                pltpu.make_async_copy(src.at[:, r, pl.ds(c, cols)],
                                      dst.at[:, r, pl.ds(c, cols)], wr_sem.at[i]).start()
            return carry
        lax.fori_loop(0, n // groups // rows, body, 0)

    write_weight(4, dwq_v, dwq_hbm, 8, 16, 512)
    write_weight(5, dwo_v, dwo_hbm, 4, 32, 512)
    write_weight(6, dw1_v, dw1_hbm, 4, 16, 1792)
    write_weight(7, dw2_v, dw2_hbm, 4, 32, 512)

    WC = W // ROWS
    for i, (src, dst) in enumerate(((dk_v, dk_hbm), (dv_v, dv_hbm))):
        for b in range(B):
            def piece(start, rows, i=i, src=src, dst=dst, b=b):
                pltpu.make_async_copy(
                    src.at[b, :, pl.ds(start, rows), :],
                    dst.at[b, :, pl.ds(Z + start, rows), :],
                    wr_sem.at[len(small) + i]).start()

            def body(j, carry, piece=piece):
                piece(pl.multiple_of(j * ROWS, ROWS), ROWS)
                return carry
            lax.fori_loop(0, WC, body, 0)
            if W > WC * ROWS:
                piece(WC * ROWS, W - WC * ROWS)

    for c in small:
        c.wait()
    for dst in (dk_hbm, dv_hbm):
        zeros = dst.at[:, :, pl.ds(0, Z), :]
        pltpu.make_async_copy(zeros, zeros, zero_sem).wait()
    for i, (src, dst) in enumerate(((dk_v, dk_hbm), (dv_v, dv_hbm))):
        pltpu.make_async_copy(
            src, dst.at[:, :, pl.ds(Z, W), :], wr_sem.at[len(small) + i]).wait()


@jax.jit
def pallas_interleave_layers__sliding_block_cached__dense_activation_gelu__decode_kernel(
    A_x: jax.Array,
    A_k_cache: jax.Array,
    A_v_cache: jax.Array,
    A_wq: jax.Array,
    A_wo: jax.Array,
    B_x: jax.Array,
    B_w1: jax.Array,
    B_b1: jax.Array,
    B_w2: jax.Array,
    B_b2: jax.Array,
    grad_out: jax.Array,
):
    del B_x
    B, HKV, SK, _ = A_k_cache.shape
    W = min(4096, max(256, SK // 4))
    R = B * (HQ // HKV)

    def like(a):
        return jax.ShapeDtypeStruct(a.shape, a.dtype)

    def vmem(a):
        return pltpu.VMEM(a.shape, a.dtype)

    window = pltpu.VMEM((B, HKV, W, DH), BF16)
    tiles = pltpu.VMEM((HKV, 2, R, DH), F32)
    hbm = pl.BlockSpec(memory_space=pltpu.HBM)
    x = A_x.reshape(B, -1)
    g = grad_out.reshape(B, -1)
    operands = (x, A_k_cache, A_v_cache, A_wq, A_wo, B_w1, B_b1, B_w2, B_b2, g)
    results = (x, x, A_k_cache, A_v_cache, A_wq, A_wo, B_w1, B_b1, B_w2, B_b2)
    out, dx, *grads = pl.pallas_call(
        _kernel,
        out_shape=[like(a) for a in results],
        in_specs=[hbm] * len(operands),
        out_specs=[hbm] * len(results),
        scratch_shapes=[
            vmem(x), vmem(g), vmem(B_b1), vmem(B_b2),
            vmem(x), vmem(x), vmem(B_b1), vmem(B_b2),
            window, window, vmem(A_wq), vmem(A_wo), vmem(B_w1), vmem(B_w2),
            window, window, vmem(A_wq), vmem(A_wo), vmem(B_w1), vmem(B_w2),
            pltpu.VMEM((HKV, ROWS, DH), BF16),
            tiles, tiles, tiles, tiles,
            pltpu.VMEM((HKV, 2, R, W), F32),
            pltpu.VMEM((HKV, R, W), F32),
            pltpu.SemaphoreType.DMA((11,)),
            pltpu.SemaphoreType.DMA(()),
            pltpu.SemaphoreType.DMA((10,)),
        ],
        compiler_params=pltpu.CompilerParams(vmem_limit_bytes=120 << 20),
    )(*operands)
    return (out.reshape(A_x.shape), dx.reshape(A_x.shape), *grads)
```

```python
import math

import jax
import jax.numpy as jnp
from jax import lax
import jax.experimental.pallas as pl
import jax.experimental.pallas.tpu as pltpu

F32 = jnp.float32
BF16 = jnp.bfloat16

HQ, DH = 32, 128
LN_EPS = 1e-5
GELU_C = math.sqrt(2.0 / math.pi)
GELU_A = 0.044715

ROWS = 112
STEP = 16
QUEUE = 64
TAIL = 512
W_ROWS = 16
W_PIECES = ((4, 512), (4, 512), (4, 896), (7, 512))

NN = (((1,), (0,)), ((), ()))
NT = (((1,), (1,)), ((), ()))
TN = (((0,), (0,)), ((), ()))


def _dot(a, b, dims):
    return lax.dot_general(a, b, dims, preferred_element_type=F32)


def _loop(lo, hi, body):
    def step(i, carry):
        body(i)
        return carry
    lax.fori_loop(lo, hi, step, 0)


def _layernorm(x):
    mean = jnp.mean(x, axis=-1, keepdims=True)
    cen = x - mean
    var = jnp.mean(cen * cen, axis=-1, keepdims=True)
    rstd = 1.0 / jnp.sqrt(var + LN_EPS)
    return cen * rstd, rstd


def _layernorm_bwd(dn, n, rstd):
    m1 = jnp.mean(dn, axis=-1, keepdims=True)
    m2 = jnp.mean(dn * n, axis=-1, keepdims=True)
    return rstd * (dn - m1 - n * m2)


def _gelu(z):
    z2 = z * z
    t = jnp.tanh(GELU_C * (z + GELU_A * z2 * z))
    cdf = 0.5 * (1.0 + t)
    dcdf = 0.5 * (1.0 - t * t) * (GELU_C * (1.0 + 3.0 * GELU_A * z2))
    return z * cdf, cdf + z * dcdf


def _kernel(
    x_hbm, k_hbm, v_hbm, wq_hbm, wo_hbm, w1_hbm, b1_hbm, w2_hbm, b2_hbm, g_hbm,
    out_hbm, dx_hbm, dk_hbm, dv_hbm, dwq_hbm, dwo_hbm, dw1_hbm, db1_hbm,
    dw2_hbm, db2_hbm,
    x_v, g_v, b1_v, b2_v, out_v, dx_v, db1_v, db2_v,
    k_v, v_v, wq_v, wo_v, w1_v, w2_v,
    dk_v, dv_v, dwq_v, dwo_v, dw1_v, dw2_v,
    zero_v, q_s, do_s, o_s, dq_s, p_s, ds_s,
    rd_sem, wr_sem, cache_sem,
):
    B, HKV, SK, _ = k_hbm.shape
    W = k_v.shape[2]
    Z = SK - W
    F = w2_hbm.shape[0]
    REP = HQ // HKV
    R = B * REP
    scale = DH ** -0.5
    caches = (dk_hbm, dv_hbm)

    reads = [
        (wq_hbm, wq_v),
        (k_hbm.at[:, :, pl.ds(Z, W), :], k_v),
        (v_hbm.at[:, :, pl.ds(Z, W), :], v_v),
        (x_hbm, x_v), (g_hbm, g_v), (b1_hbm, b1_v), (b2_hbm, b2_v),
        (wo_hbm, wo_v), (w1_hbm, w1_v),
        (w2_hbm.at[pl.ds(0, F - TAIL)], w2_v.at[pl.ds(0, F - TAIL)]),
        (w2_hbm.at[pl.ds(F - TAIL, TAIL)], w2_v.at[pl.ds(F - TAIL, TAIL)]),
    ]
    reads = [pltpu.make_async_copy(src, dst, rd_sem.at[i])
             for i, (src, dst) in enumerate(reads)]
    for copy in reads:
        copy.start()
    zero_v[...] = jnp.zeros(zero_v.shape, zero_v.dtype)
    for copy in reads[:-1]:
        copy.wait()

    ZC = Z // ROWS
    NZ = B * ZC
    assert Z % ROWS == 0 and NZ % STEP == 0

    def fill_cache(i, first, n):
        def start(j):
            rows = pl.ds(pl.multiple_of((j % ZC) * ROWS, ROWS), ROWS)
            pltpu.make_async_copy(
                zero_v, caches[i].at[j // ZC, :, rows, :], cache_sem.at[i]).start()
        _loop(first, first + n, start)

    issued = 0

    def top_up(n=STEP):
        nonlocal issued
        assert issued + n <= 2 * NZ
        while n:
            m = min(n, NZ - issued % NZ)
            fill_cache(issued // NZ, issued % NZ, m)
            issued += m
            n -= m

    def head_loop(body, n=STEP):
        nonlocal issued
        base = issued
        assert base % STEP == 0 and n % STEP == 0 and base + HKV * n <= 2 * NZ

        def step(h):
            for off in range(0, n, STEP):
                first = base + h * n + off
                pl.when(first < NZ)(lambda: fill_cache(0, first, STEP))
                pl.when(first >= NZ)(lambda: fill_cache(1, first - NZ, STEP))
            body(h)
        _loop(0, HKV, step)
        issued = base + HKV * n

    top_up(QUEUE)
    reads[-1].wait()

    def row_ids(width):
        return lax.broadcasted_iota(jnp.int32, (R, width), 0)

    def per_batch(fn):
        y = fn(0)
        for b in range(1, B):
            y = jnp.where(row_ids(y.shape[1]) % B == b, fn(b), y)
        return y

    def load_rows(ref):
        x = ref[...].astype(F32)
        return per_batch(lambda b: jnp.broadcast_to(x[b:b + 1], (R, x.shape[1])))

    def split_heads(x, ref, layer):
        head = row_ids(DH) // B
        for h in range(HKV):
            cols = [x[:, c * DH:(c + 1) * DH] for c in range(h * REP, (h + 1) * REP)]
            tile = cols[0]
            for r in range(1, REP):
                tile = jnp.where(head == r, cols[r], tile)
            ref[h, layer] = tile

    def merge_heads(ref, layer):
        head = row_ids(DH) // B
        cols = []
        for h in range(HKV):
            tile = ref[h, layer]
            for r in range(REP):
                col = jnp.where(head == r, tile, 0.0)
                shift = B
                while shift < R:
                    col = col + pltpu.roll(col, shift, axis=0)
                    shift *= 2
                cols.append(col)
        return jnp.concatenate(cols, axis=1)

    def distinct_rows(a):
        return jnp.where(row_ids(a.shape[1]) < B, a, 0.0)

    def weight_grad(ref, a0, a1, b0, b1):
        a = jnp.concatenate([distinct_rows(a0), distinct_rows(a1)], axis=0)
        b = jnp.concatenate([b0, b1], axis=0)
        grad = _dot(a.astype(BF16), b.astype(BF16), TN)
        ref[...] = grad.astype(BF16).reshape(ref.shape)

    def bias_grad(ref, a0, a1):
        grad = jnp.sum(distinct_rows(a0 + a1), axis=0, keepdims=True)
        ref[...] = grad.reshape(-1).astype(BF16)

    def attn_fwd(x, layer):
        n, rstd = _layernorm(x)
        split_heads(_dot(n.astype(BF16), wq_v[...], NN), q_s, layer)
        top_up()

        def body(h):
            q = q_s[h, layer].astype(BF16)
            s = per_batch(lambda b: _dot(q, k_v[b, h], NT)) * scale
            e = jnp.exp(s - jnp.max(s, axis=-1, keepdims=True))
            p = e / jnp.sum(e, axis=-1, keepdims=True)
            p_s[h, layer] = p
            pb = p.astype(BF16)
            o_s[h, layer] = per_batch(lambda b: _dot(pb, v_v[b, h], NN))
        head_loop(body)
        o = merge_heads(o_s, layer)
        y = _dot(o.astype(BF16), wo_v[...], NN)
        top_up()
        return x + y, n, rstd, o

    def attn_bwd(g, layer, n, rstd):
        split_heads(_dot(g.astype(BF16), wo_v[...], NT), do_s, layer)
        top_up()

        def body(h):
            do = do_s[h, layer].astype(BF16)
            dp = per_batch(lambda b: _dot(do, v_v[b, h], NT))
            p = p_s[h, layer]
            ds = p * (dp - jnp.sum(p * dp, axis=-1, keepdims=True)) * scale
            dsb = ds.astype(BF16)
            dq_s[h, layer] = per_batch(lambda b: _dot(dsb, k_v[b, h], NN))
            if layer == 1:
                ds_s[h] = ds
                return

            batch = lax.broadcasted_iota(jnp.int32, (2 * R, DH), 0) % B

            def window_grad(dst, a0, a1, tiles):
                a = jnp.concatenate([a0, a1], axis=0)
                t = jnp.concatenate([tiles[h, 0], tiles[h, 1]], axis=0)
                t = jnp.concatenate(
                    [jnp.where(batch == b, t, 0.0) for b in range(B)], axis=1)
                grad = _dot(a.astype(BF16), t.astype(BF16), TN)
                for b in range(B):
                    dst[b, h] = grad[:, b * DH:(b + 1) * DH].astype(BF16)

            window_grad(dk_v, ds, ds_s[h], q_s)
            window_grad(dv_v, p, p_s[h, 1], do_s)
        head_loop(body, STEP if layer == 1 else 2 * STEP)
        dq = merge_heads(dq_s, layer)
        dn = _dot(dq.astype(BF16), wq_v[...], NT)
        top_up()
        return g + _layernorm_bwd(dn, n, rstd), dq

    def ffn_fwd(x):
        n, rstd = _layernorm(x)
        b1 = b1_v[...].astype(F32).reshape(1, -1)
        b2 = b2_v[...].astype(F32).reshape(1, -1)
        a, da = _gelu(_dot(n.astype(BF16), w1_v[...], NN) + b1)
        y = _dot(a.astype(BF16), w2_v[...], NN) + b2
        return x + y, n, rstd, a, da

    def ffn_bwd(g, n, rstd, da):
        dz = _dot(g.astype(BF16), w2_v[...], NT) * da
        dn = _dot(dz.astype(BF16), w1_v[...], NT)
        return g + _layernorm_bwd(dn, n, rstd), dz

    x0 = load_rows(x_v)
    x1, n0, r0, o0 = attn_fwd(x0, 0)
    x2, n1, r1, a0, da0 = ffn_fwd(x1)
    x3, n2, r2, o1 = attn_fwd(x2, 1)
    x4, n3, r3, a1, da1 = ffn_fwd(x3)
    out_v[...] = x4[:B].astype(BF16)

    g4 = load_rows(g_v)
    g3, dz1 = ffn_bwd(g4, n3, r3, da1)
    g2, dq1 = attn_bwd(g3, 1, n2, r2)
    g1, dz0 = ffn_bwd(g2, n1, r1, da0)
    g0, dq0 = attn_bwd(g1, 0, n0, r0)
    dx_v[...] = g0[:B].astype(BF16)

    bias_grad(db1_v, dz0, dz1)
    bias_grad(db2_v, g2, g4)
    weight_grad(dwq_v, n0, n2, dq0, dq1)
    weight_grad(dwo_v, o0, o1, g1, g3)
    weight_grad(dw1_v, n1, n3, dz0, dz1)
    weight_grad(dw2_v, a0, a1, g2, g4)

    writes = [
        (dwq_v, dwq_hbm), (dwo_v, dwo_hbm), (dw1_v, dw1_hbm), (dw2_v, dw2_hbm),
        (out_v, out_hbm), (dx_v, dx_hbm), (db1_v, db1_hbm), (db2_v, db2_hbm),
    ]
    whole = [pltpu.make_async_copy(src, dst, wr_sem.at[i])
             for i, (src, dst) in enumerate(writes)]
    for copy in whole[4:]:
        copy.start()
    top_up(2 * NZ - issued)

    def weight_pieces(i):
        src, dst = writes[i]
        cols = W_PIECES[i][1]
        _, n, m = src.shape
        assert n % W_ROWS == 0 and m % cols == 0
        per_row = m // cols

        def start(j):
            r = pl.ds(pl.multiple_of((j // per_row) * W_ROWS, W_ROWS), W_ROWS)
            c = pl.ds(pl.multiple_of((j % per_row) * cols, cols), cols)
            pltpu.make_async_copy(
                src.at[:, r, c], dst.at[:, r, c], wr_sem.at[i]).start()
        return n // W_ROWS * per_row, start

    for i in (0, 2):
        (count, first), (other, second) = weight_pieces(i), weight_pieces(i + 1)
        assert count == other
        _loop(0, count, lambda j: (first(j), second(j)))

    for i, src in enumerate((dk_v, dv_v)):
        for b in range(B):
            def start(row, rows):
                pltpu.make_async_copy(
                    src.at[b, :, pl.ds(row, rows), :],
                    caches[i].at[b, :, pl.ds(Z + row, rows), :],
                    cache_sem.at[i]).start()
            _loop(0, W // ROWS,
                  lambda j: start(pl.multiple_of(j * ROWS, ROWS), ROWS))
            if W % ROWS:
                start(W - W % ROWS, W % ROWS)

    for copy in whole:
        copy.wait()
    for i, cache in enumerate(caches):
        pltpu.make_async_copy(cache, cache, cache_sem.at[i]).wait()


@jax.jit
def pallas_interleave_layers__sliding_block_cached__dense_activation_gelu__decode_kernel(
    A_x: jax.Array,
    A_k_cache: jax.Array,
    A_v_cache: jax.Array,
    A_wq: jax.Array,
    A_wo: jax.Array,
    B_x: jax.Array,
    B_w1: jax.Array,
    B_b1: jax.Array,
    B_w2: jax.Array,
    B_b2: jax.Array,
    grad_out: jax.Array,
):
    del B_x
    B, HKV, SK, _ = A_k_cache.shape
    W = min(4096, max(256, SK // 4))
    R = B * (HQ // HKV)

    x = A_x.reshape(B, -1)
    g = grad_out.reshape(B, -1)
    weights = (A_wq, A_wo, B_w1, B_w2)
    dwq, dwo, dw1, dw2 = (
        (groups, w.shape[0] // groups, w.shape[1])
        for w, (groups, _) in zip(weights, W_PIECES))

    operands = (x, A_k_cache, A_v_cache, A_wq, A_wo, B_w1, B_b1, B_w2, B_b2, g)
    out_shapes = (x.shape, x.shape, A_k_cache.shape, A_v_cache.shape,
                  dwq, dwo, dw1, B_b1.shape, dw2, B_b2.shape)
    vectors = (x.shape, x.shape, B_b1.shape, B_b2.shape)
    window = (B, HKV, W, DH)
    buffers = (*vectors, *vectors,
               window, window, *(w.shape for w in weights),
               window, window, dwq, dwo, dw1, dw2,
               (HKV, ROWS, DH))
    tiles = pltpu.VMEM((HKV, 2, R, DH), F32)
    hbm = pl.BlockSpec(memory_space=pltpu.HBM)

    results = pl.pallas_call(
        _kernel,
        out_shape=[jax.ShapeDtypeStruct(s, BF16) for s in out_shapes],
        in_specs=[hbm] * len(operands),
        out_specs=[hbm] * len(out_shapes),
        scratch_shapes=[
            *(pltpu.VMEM(s, BF16) for s in buffers),
            tiles, tiles, tiles, tiles,
            pltpu.VMEM((HKV, 2, R, W), F32),
            pltpu.VMEM((HKV, R, W), F32),
            pltpu.SemaphoreType.DMA((11,)),
            pltpu.SemaphoreType.DMA((8,)),
            pltpu.SemaphoreType.DMA((2,)),
        ],
        compiler_params=pltpu.CompilerParams(vmem_limit_bytes=120 << 20),
    )(*operands)

    like = (A_x, A_x, A_k_cache, A_v_cache, A_wq, A_wo, B_w1, B_b1, B_w2, B_b2)
    return tuple(r.reshape(a.shape) for r, a in zip(results, like))
```
